```python
import os as _os
_os.environ.setdefault("JAX_PLATFORMS", "cpu")
import jax
import jax.numpy as jnp

def _softmax(x, axis=-1):
    return jax.nn.softmax(x, axis=axis)
def _gelu(x):
    return jax.nn.gelu(x, approximate=True)
def _silu(x):
    return jax.nn.silu(x)
def _sigmoid(x):
    return jax.nn.sigmoid(x)
def _layernorm(x, axis=-1, eps=1e-5):
    m = jnp.mean(x, axis=axis, keepdims=True)
    v = jnp.var(x, axis=axis, keepdims=True)
    return (x - m) / jnp.sqrt(v + eps)
def _scatter_add(tgt, idx, src, axis=0):
    return tgt.at[idx].add(src)
def _segment_sum(src, seg, n):
    return jax.ops.segment_sum(src, seg, n)
class _Rng:
    def __init__(self, key):
        self._k = key
    def _next(self):
        self._k, sub = jax.random.split(self._k)
        return sub
    def normal(self, shape):
        return jax.random.normal(self._next(), shape, dtype=jnp.bfloat16)
    def randint(self, lo, hi, shape):
        return jax.random.randint(self._next(), shape, lo, hi, dtype=jnp.int32)
    def uniform(self, shape, lo=0.0, hi=1.0):
        return jax.random.uniform(self._next(), shape, jnp.bfloat16, lo, hi)
    def permutation(self, n):
        return jax.random.permutation(self._next(), n)


kernel_name = 'concat_heads__softmax_full_mha__softmax_full_mha__prompt'

def setup_inputs():
    _rng = _Rng(jax.random.key(int.from_bytes(__import__("os").urandom(4), "little")))
    _w = (lambda a: (lambda t: t.astype(jnp.bfloat16) if jnp.issubdtype(t.dtype, jnp.floating) else t)(jnp.asarray(a)))
    def _A_setup():
        B, S, D = 1, 2048, 512
        return {
            "x": _w((lambda *s: _rng.normal(s) * 0.2)(B, S, D)),
            "wqkv": _w((lambda *s: _rng.normal(s) * 0.2)(D, 3 * D)),
            "wo": _w((lambda *s: _rng.normal(s) * 0.05)(D, D)),
        }
    _A_in = _A_setup()

    def _B_setup():
        B, S, D = 1, 2048, 512
        return {
            "x": _w((lambda *s: _rng.normal(s) * 0.2)(B, S, D)),
            "wqkv": _w((lambda *s: _rng.normal(s) * 0.2)(D, 3 * D)),
            "wo": _w((lambda *s: _rng.normal(s) * 0.05)(D, D)),
        }
    _B_in = _B_setup()

    return {
        "A_x": _A_in["x"],
        "A_wqkv": _A_in["wqkv"],
        "A_wo": _A_in["wo"],
        "B_x": _B_in["x"],
        "B_wqkv": _B_in["wqkv"],
        "B_wo": _B_in["wo"],
    }

def reference(A_x, A_wqkv, A_wo, B_x, B_wqkv, B_wo):
    def _A_ref(x, wqkv, wo):
        B, S, D = x.shape
        H = 32; Dh = D // H
        qkv = (lambda x, *d: x.transpose(*d))((x @ wqkv).reshape(B, S, 3, H, Dh), 2, 0, 3, 1, 4)
        q, k, v = qkv[0], qkv[1], qkv[2]
        scale = Dh ** -0.5
        scores = jnp.einsum("bhqd,bhkd->bhqk", q, k) * scale
        p = _softmax(scores, axis=-1)
        o = jnp.einsum("bhqk,bhkd->bhqd", p, v)
        return (lambda x, *d: x.transpose(*d))(o, 0, 2, 1, 3).reshape(B, S, D) @ wo

    def _B_ref(x, wqkv, wo):
        B, S, D = x.shape
        H = 32; Dh = D // H
        qkv = (lambda x, *d: x.transpose(*d))((x @ wqkv).reshape(B, S, 3, H, Dh), 2, 0, 3, 1, 4)
        q, k, v = qkv[0], qkv[1], qkv[2]
        scale = Dh ** -0.5
        scores = jnp.einsum("bhqd,bhkd->bhqk", q, k) * scale
        p = _softmax(scores, axis=-1)
        o = jnp.einsum("bhqk,bhkd->bhqd", p, v)
        return (lambda x, *d: x.transpose(*d))(o, 0, 2, 1, 3).reshape(B, S, D) @ wo

    a = _A_ref(A_x, A_wqkv, A_wo)
    b = _B_ref(B_x, B_wqkv, B_wo)
    return jnp.concatenate([a, b], axis=-1)
```

```python
import functools
import math

import jax
import jax.numpy as jnp
from jax import lax
import jax.experimental.pallas as pl
import jax.experimental.pallas.tpu as pltpu

S = 2048
D = 512
H = 32
DH = 16
TQ = 128
CH = 128
LAG = 10
LOG2E = math.log2(math.e)
QSCALE = (DH ** -0.5) * LOG2E
FAST_BOUND = 40.0
BF = jnp.bfloat16
F32 = jnp.float32
U32 = jnp.uint32


def _pack(x):
    return pltpu.bitcast(x, U32)


def _unpack(x):
    return pltpu.bitcast(x, BF)


def _kernel(ax, aw, ao, bx, bw, bo, out_hbm,
            x_buf, w_buf, wo_buf, wt_s, k_s, qt_s, vt_s, ot_s, s_s, out_buf, in_sem, out_sem):
    srcs = ((ax, aw, ao), (bx, bw, bo))
    def in_copies(p):
        x, w, o = srcs[p]
        return (pltpu.make_async_copy(w, w_buf.at[p], in_sem.at[p, 0]),
                pltpu.make_async_copy(x.at[0], x_buf.at[p], in_sem.at[p, 1]),
                pltpu.make_async_copy(o, wo_buf.at[p], in_sem.at[p, 2]))
    for p in range(2):
        for c in in_copies(p):
            c.start()

    def out_copy(p, r0, n):
        return pltpu.make_async_copy(
            out_buf.at[p, pl.ds(r0, n), :],
            out_hbm.at[0, pl.ds(r0, n), pl.ds(pl.multiple_of(p * D, D), D)],
            out_sem.at[p])

    def problem(p, carry):
        pltpu.make_async_copy(aw, w_buf.at[p], in_sem.at[p, 0]).wait()
        for i, c0 in enumerate((0, 2 * D)):
            w = w_buf[p, :, c0:c0 + D]
            wt_s[i * D:(i + 1) * D, :] = w.astype(F32).T.astype(BF)
        pltpu.make_async_copy(ax.at[0], x_buf.at[p], in_sem.at[p, 1]).wait()

        PB = 256
        def proj(i, c):
            kmax, qmax, vmax = c
            r0 = pl.multiple_of(i * PB, PB)
            xb = x_buf[p, pl.ds(r0, PB), :]
            k = jnp.dot(xb, w_buf[p, :, D:2 * D], preferred_element_type=F32)
            kb = k.astype(BF)
            k_s[pl.ds(pl.multiple_of(i * (PB // 2), PB // 2), PB // 2), :] = _pack(kb)
            qv = lax.dot_general(wt_s[...], xb, (((1,), (1,)), ((), ())),
                                 preferred_element_type=F32)
            qb = (qv[:D] * QSCALE).astype(BF)
            vb = qv[D:].astype(BF)
            qt_s[:, pl.ds(r0, PB)] = _pack(qb)
            vt_s[:, pl.ds(r0, PB)] = _pack(vb)
            rows = lax.broadcasted_iota(jnp.int32, (H, D), 0)
            cols = lax.broadcasted_iota(jnp.int32, (H, D), 1)
            e = jnp.where(cols // DH == rows, 1.0, 0.0).astype(BF)
            qf = qb.astype(F32)
            kf = kb.astype(F32)
            qn = jnp.dot(e, (qf * qf).astype(BF), preferred_element_type=F32)
            kn = lax.dot_general(e, (kf * kf).astype(BF), (((1,), (1,)), ((), ())),
                                 preferred_element_type=F32)
            va = jnp.abs(vb.astype(F32)).reshape(D // 8, 8, PB).max(axis=0)
            return (jnp.maximum(kmax, kn), jnp.maximum(qmax, qn), jnp.maximum(vmax, va))
        z = jnp.zeros((H, PB), F32)
        kmax, qmax, vmax = lax.fori_loop(0, S // PB, proj, (z, z, jnp.zeros((8, PB), F32)))
        kq = jnp.max(kmax, axis=1, keepdims=True) * jnp.max(qmax, axis=1, keepdims=True)
        bound2 = jnp.max(kq) * 1.05
        vm = jnp.max(vmax)
        fast = jnp.logical_and(bound2 <= FAST_BOUND * FAST_BOUND,
                               jnp.logical_and(vm <= 2.0 ** 60, vm >= 2.0 ** -60))

        def weights(h, q0):
            qv = _unpack(qt_s[pl.ds(h * 8, 8), pl.ds(q0, TQ)])
            z = jnp.zeros((DH, TQ), BF)
            return jnp.concatenate([qv if i == h % 8 else z for i in range(8)], axis=0)

        @pl.when(fast)
        def _():
            NCH = S // CH
            def body(j, c):
                q0 = pl.multiple_of(j * TQ, TQ)
                items = [(h, c) for h in range(H) for c in range(NCH)]
                ws = {}; ps = {}; acc = {}; l = {}
                def qk(h, c):
                    if h not in ws:
                        ws[h] = weights(h, q0)
                    g = h // 8
                    kk = _unpack(k_s[c * CH // 2:(c + 1) * CH // 2, g * 128:(g + 1) * 128])
                    s = jnp.dot(kk, ws[h], preferred_element_type=F32)
                    e = jnp.exp2(s)
                    ls = e.reshape(CH // 8, 8, TQ).sum(axis=0)
                    l[h] = ls if h not in l else l[h] + ls
                    ps[(h, c)] = e.astype(BF)
                def pv(h, c):
                    vv = _unpack(vt_s[h * 8:(h + 1) * 8, c * CH:(c + 1) * CH])
                    o = jnp.dot(vv, ps.pop((h, c)), preferred_element_type=F32)
                    acc[h] = o if h not in acc else acc[h] + o
                    if c == NCH - 1:
                        lsum = l[h].sum(axis=0, keepdims=True)
                        ot_s[h * 8:(h + 1) * 8, pl.ds(q0, TQ)] = _pack((acc[h] / lsum).astype(BF))
                for i in range(len(items) + LAG):
                    if i < len(items):
                        qk(*items[i])
                    if i >= LAG:
                        pv(*items[i - LAG])
                return c
            lax.fori_loop(0, S // TQ, body, 0)

        @pl.when(jnp.logical_not(fast))
        def _():
            def body(it, c):
                j = it // (H // 8)
                g = it % (H // 8)
                q0 = pl.multiple_of(j * TQ, TQ)
                l0 = pl.multiple_of(g * 128, 128)
                for hh in range(8):
                    r0 = pl.multiple_of((g * 8 + hh) * 8, 8)
                    qv = _unpack(qt_s[pl.ds(r0, 8), pl.ds(q0, TQ)])
                    z = jnp.zeros((DH, TQ), BF)
                    w = jnp.concatenate([qv if i == hh else z for i in range(8)], axis=0)
                    s_s[...] = jnp.dot(_unpack(k_s[:, pl.ds(l0, 128)]), w, preferred_element_type=F32)
                    m = jnp.max(s_s[...], axis=0, keepdims=True)
                    e = jnp.exp2(s_s[...] - m)
                    lsum = jnp.sum(e, axis=0, keepdims=True)
                    o = jnp.dot(_unpack(vt_s[pl.ds(r0, 8), :]), e.astype(BF), preferred_element_type=F32)
                    ot_s[pl.ds(r0, 8), pl.ds(q0, TQ)] = _pack((o / lsum).astype(BF))
                return c
            lax.fori_loop(0, (S // TQ) * (H // 8), body, 0)

        pltpu.make_async_copy(ao, wo_buf.at[p], in_sem.at[p, 2]).wait()
        OB = 256
        def oproj(i, c):
            r0 = pl.multiple_of(i * OB, OB)
            ot = _unpack(ot_s[:, pl.ds(r0, OB)])
            o = ot.astype(F32).T.astype(BF)
            out_buf[p, pl.ds(r0, OB), :] = jnp.dot(o, wo_buf[p], preferred_element_type=F32).astype(BF)
            out_copy(p, r0, OB).start()
            return c
        lax.fori_loop(0, S // OB, oproj, 0)
        return carry

    lax.fori_loop(0, 2, problem, 0)
    for p in range(2):
        out_copy(p, 0, S).wait()


@jax.jit
def pallas_concat_heads__softmax_full_mha__softmax_full_mha__prompt_kernel(
    A_x: jax.Array,
    A_wqkv: jax.Array,
    A_wo: jax.Array,
    B_x: jax.Array,
    B_wqkv: jax.Array,
    B_wo: jax.Array,
):
    any_spec = pl.BlockSpec(memory_space=pl.ANY)
    return pl.pallas_call(
        _kernel,
        out_shape=jax.ShapeDtypeStruct((1, S, 2 * D), BF),
        in_specs=[any_spec] * 6,
        out_specs=any_spec,
        scratch_shapes=[
            pltpu.VMEM((2, S, D), BF),
            pltpu.VMEM((2, D, 3 * D), BF),
            pltpu.VMEM((2, D, D), BF),
            pltpu.VMEM((2 * D, D), BF),
            pltpu.VMEM((S // 2, D), U32),
            pltpu.VMEM((D // 2, S), U32),
            pltpu.VMEM((D // 2, S), U32),
            pltpu.VMEM((D // 2, S), U32),
            pltpu.VMEM((S, TQ), F32),
            pltpu.VMEM((2, S, D), BF),
            pltpu.SemaphoreType.DMA((2, 3)),
            pltpu.SemaphoreType.DMA((2,)),
        ],
        compiler_params=pltpu.CompilerParams(vmem_limit_bytes=100 * 1024 * 1024),
        name="mha2",
    )(A_x, A_wqkv, A_wo, B_x, B_wqkv, B_wo)
```

```python
import math

import jax
import jax.numpy as jnp
from jax import lax
import jax.experimental.pallas as pl
import jax.experimental.pallas.tpu as pltpu

S = 2048
D = 512
H = 32
DH = 16
TQ = 128
NT = S // TQ
NU = 2
CH = 256
PT = 128
LT = 13
XCH = (256, 768, 1024)
GS = 2
QSCALE = (DH ** -0.5) * math.log2(math.e)
NREP = 6
USPLIT = 6.0
AMAX = 127.0 * (1.0 - 2.0 ** -12)
MAGIC = 1.5 * 2.0 ** 23
RANGE_BOUND = 60.0
PREC_BOUND = 16.0
TINY = 1e-30
BF = jnp.bfloat16
F32 = jnp.float32
I32 = jnp.int32
I8 = jnp.int8
U32 = jnp.uint32
NT_DIMS = (((1,), (1,)), ((), ()))


def _limbs(a):
    th = a + MAGIC
    r = a - (th - MAGIC)
    tu = a * (1.0 / USPLIT) + MAGIC
    tl = r * (NREP * USPLIT) + MAGIC
    return tuple(lax.bitcast_convert_type(t, I32) for t in (th, tu, tl))


def _reduce_rows(xs, op, sub):
    for sh in (1, 2, 4):
        if len(xs) > 1:
            m = (sub & sh) == 0
            xs = [op(jnp.where(m, a, b), pltpu.roll(jnp.where(m, b, a), sh, 0))
                  for a, b in zip(xs[0::2], xs[1::2])]
        else:
            xs = [op(xs[0], pltpu.roll(xs[0], sh, 0))]
    return xs[0]


def _kernel(ax, aw, ao, bx, bw, bo, out_hbm,
            x_buf, w_buf, wo_buf, wt_s, kf_s, kcol_s, k8_s, q8_s, sc_s, vt_s, ot_s,
            qt_s, s_s, out_buf, w_sem, x_sem, out_sem):
    xoff = [sum(XCH[:i]) for i in range(len(XCH))]

    def w_copy(w, p, part):
        cols = pl.ds(part * D, D)
        return pltpu.make_async_copy(w.at[:, cols], w_buf.at[p, :, cols], w_sem.at[p, part])

    def wo_copy(o, p):
        return pltpu.make_async_copy(o, wo_buf.at[p], w_sem.at[p, 3])

    def x_copy(x, p, i):
        rows = pl.ds(xoff[i], XCH[i])
        return pltpu.make_async_copy(x.at[0, rows, :], x_buf.at[p, rows, :], x_sem.at[p, i])

    def out_copy(p, r0, n):
        return pltpu.make_async_copy(
            out_buf.at[p, pl.ds(r0, n), :],
            out_hbm.at[0, pl.ds(r0, n), pl.ds(pl.multiple_of(p * D, D), D)],
            out_sem.at[p])

    w_copy(aw, 0, 1).start()
    x_copy(ax, 0, 0).start()
    x_copy(ax, 0, 1).start()
    ot_s[NU - 1] = jnp.zeros((D, TQ), F32)

    def problem(p, carry):
        w_copy(aw, p, 1).wait()
        kmax = jnp.full((8, D), TINY, F32)
        for i in range(len(XCH)):
            x_copy(ax, p, i).wait()

            @pl.when(p == 0)
            def _():
                if i + 2 < len(XCH):
                    x_copy(ax, 0, i + 2).start()
                if i == len(XCH) - 3 or (len(XCH) < 3 and i == 0):
                    w_copy(aw, 0, 0).start()
                if i == len(XCH) - 2:
                    w_copy(aw, 0, 2).start()
                if i == len(XCH) - 1:
                    wo_copy(ao, 0).start()
                    for part in (1, 0, 2):
                        w_copy(bw, 1, part).start()
                    for c in range(len(XCH)):
                        x_copy(bx, 1, c).start()
                    wo_copy(bo, 1).start()

            if i == len(XCH) - 1:
                w_copy(aw, p, 0).wait()
            rows = slice(xoff[i], xoff[i] + XCH[i])
            k = jnp.dot(x_buf[p, rows, :], w_buf[p, :, D:2 * D], preferred_element_type=F32)
            kf_s[rows, :] = k
            kmax = jnp.maximum(kmax, jnp.abs(k).reshape(XCH[i] // 8, 8, D).max(axis=0))
        wt_s[0:D // 2, :] = pltpu.bitcast(w_buf[p, :, 0:D].astype(F32).T.astype(BF), U32)
        w_copy(aw, p, 2).wait()
        wt_s[D // 2:D, :] = pltpu.bitcast(w_buf[p, :, 2 * D:3 * D].astype(F32).T.astype(BF), U32)

        kmax = jnp.max(kmax, axis=0, keepdims=True)
        kinv = 127.0 / kmax
        kcol_s[...] = jnp.broadcast_to(kmax * QSCALE, (128, D)).T

        lane_blk = lax.broadcasted_iota(I32, (8, 128), 1) // DH
        masks = [(lane_blk & (1 << b)) != 0 for b in range(3)]
        sub = lax.broadcasted_iota(I32, (8, 128), 0)

        qsm = l1m = vmax = jnp.zeros((8, 128), F32)
        for n in range(NT):
            cols = slice(n * 128, (n + 1) * 128)
            q = lax.dot_general(pltpu.bitcast(wt_s[0:D // 2, :], BF), x_buf[p, cols, :],
                                NT_DIMS, preferred_element_type=F32)
            for g in range(H // GS):
                rows = slice(g * GS * DH, (g + 1) * GS * DH)
                qp = q[rows] * kcol_s[rows, :]
                aq = jnp.abs(qp)
                lo = [aq[h * DH:h * DH + 8] for h in range(GS)]
                hi = [aq[h * DH + 8:(h + 1) * DH] for h in range(GS)]
                qs = _reduce_rows([jnp.maximum(a, b) for a, b in zip(lo, hi)], jnp.maximum, sub)
                l1 = _reduce_rows([a + b for a, b in zip(lo, hi)], jnp.add, sub)
                qsm = jnp.maximum(qsm, qs)
                l1m = jnp.maximum(l1m, l1)
                qs = jnp.maximum(qs, TINY)
                r = pl.reciprocal(qs, approx=True)
                r = r * (2.0 - qs * r) * AMAX
                sc_s[g * GS:(g + 1) * GS, cols] = (qs * (1.0 / (NREP * AMAX * 127.0)))[0:GS]
                for u in range(GS):
                    h = g * GS + u
                    ah, au, al = _limbs(qp[u * DH:(u + 1) * DH] * r[u:u + 1, :])
                    blocks = []
                    for j in range(8):
                        rr = (j - h) % 8
                        blocks.append(ah if rr < NREP else (au if rr == NREP else al))
                    w8 = jnp.concatenate(blocks, axis=0).astype(I8)
                    q8_s[h, :, cols] = pltpu.bitcast(w8, U32)
        for n in range(NT):
            cols = slice(n * 128, (n + 1) * 128)
            v = lax.dot_general(pltpu.bitcast(wt_s[D // 2:D, :], BF), x_buf[p, cols, :],
                                NT_DIMS, preferred_element_type=F32)
            vt_s[:, cols] = pltpu.bitcast(v.astype(BF), U32)
            vmax = jnp.maximum(vmax, jnp.abs(v).reshape(D // 8, 8, 128).max(axis=0))
            bh, bu, bl = [pltpu.bitcast(t.astype(I8), U32)
                          for t in _limbs(kf_s[cols, :] * kinv)]
            for g in range(D // 128):
                pieces = []
                for t in range(4):
                    ys = []
                    for r in range(8):
                        src = bh if r < NREP else (bl if r == NREP else bu)
                        y = src[t * 8:(t + 1) * 8, g * 128:(g + 1) * 128]
                        ys.append(pltpu.roll(y, DH * r, 1) if r else y)
                    for b in range(3):
                        ys = [jnp.where(masks[b], ys[(m + (1 << b)) % 8], ys[m]) for m in range(8)]
                    pieces.append(ys)
                for pos in range(8):
                    k8_s[g * 8 + pos, n * 32:(n + 1) * 32, :] = jnp.concatenate(
                        [ys[(8 - pos) % 8] for ys in pieces], axis=0)
        vm = jnp.max(vmax)
        worst = jnp.max(jnp.maximum(l1m * (1.0 / RANGE_BOUND), qsm * (1.0 / PREC_BOUND)))
        fast = jnp.logical_and(worst <= 1.0, jnp.logical_and(vm <= 2.0 ** 40, vm >= 2.0 ** -40))
        wo_copy(ao, p).wait()

        def o_natural(slot):
            return ot_s[slot].T.astype(BF)

        def oproj(o, r0):
            for n in range(D // 128):
                out_buf[p, pl.ds(r0, TQ), n * 128:(n + 1) * 128] = jnp.dot(
                    o, wo_buf[p, :, n * 128:(n + 1) * 128], preferred_element_type=F32).astype(BF)

        @pl.when(fast)
        def _():
            NCH = S // CH
            TPC = CH // PT
            PER = PT // 32
            order = [t * PER + (PER - 1 - i) for t in range(TPC) for i in range(PER)]
            inv = {b: i for i, b in enumerate(order)}

            def body(j, c):
                q0s = [pl.multiple_of((NU * j + u) * TQ, TQ) for u in range(NU)]
                prev0 = pl.multiple_of(((NU * j + NT - 1) % NT) * TQ, TQ)
                o_prev = o_natural(NU - 1)
                items = [(u, h, c) for u in range(NU) for h in range(H) for c in range(NCH)]
                tiles = [(u, h, t) for u in range(NU) for h in range(H) for t in range(S // PT)]
                ws = {}; ps = {}; acc = {}; l = {}
                def qk(u, h, c):
                    if (u, h) not in ws:
                        ws[(u, h)] = (pltpu.bitcast(q8_s[h, :, pl.ds(q0s[u], TQ)], I8),
                                      sc_s[h:h + 1, pl.ds(q0s[u], TQ)])
                    w, sc = ws[(u, h)]
                    kk = k8_s[h, c * CH // 4:(c + 1) * CH // 4, :]
                    kk = jnp.concatenate([kk[b * 8:(b + 1) * 8] for b in order], axis=0)
                    a = jnp.dot(pltpu.bitcast(kk, I8), w, preferred_element_type=I32)
                    e = jnp.exp2(a.astype(F32) * sc)
                    ls = e.reshape(CH // 8, 8, TQ).sum(axis=0)
                    l[(u, h)] = ls if (u, h) not in l else l[(u, h)] + ls
                    for t in range(TPC):
                        et = jnp.concatenate([e[inv[b] * 32:(inv[b] + 1) * 32]
                                              for b in range(t * PER, (t + 1) * PER)], axis=0)
                        ps[(u, h, c * TPC + t)] = et.astype(BF)
                def pv(u, h, t):
                    vv = pltpu.bitcast(vt_s[h * 8:(h + 1) * 8, t * PT:(t + 1) * PT], BF)
                    o = jnp.dot(vv, ps.pop((u, h, t)), preferred_element_type=F32)
                    acc[(u, h)] = o if (u, h) not in acc else acc[(u, h)] + o
                    if t == S // PT - 1:
                        lsum = l[(u, h)].sum(axis=0, keepdims=True)
                        ot_s[u, h * DH:(h + 1) * DH, :] = acc[(u, h)] / lsum
                nt = 0
                per_u = H * NCH
                for i in range(len(items)):
                    qk(*items[i])
                    if i == 16:
                        oproj(o_prev, prev0)
                    for u in range(NU - 2):
                        if i == (u + 1) * per_u + 16:
                            oproj(o_natural(u), q0s[u])
                    if i == len(items) - 1:
                        oproj(o_natural(NU - 2), q0s[NU - 2])
                    while nt < TPC * (i + 1) - LT:
                        pv(*tiles[nt]); nt += 1
                while nt < len(tiles):
                    pv(*tiles[nt]); nt += 1

                @pl.when(j > 0)
                def _():
                    out_copy(p, prev0, TQ).start()
                out_copy(p, q0s[0], (NU - 1) * TQ).start()
                return c
            with jax.named_scope('attn'):
                lax.fori_loop(0, NT // NU, body, 0)
            oproj(o_natural(NU - 1), S - TQ)
            out_copy(p, S - TQ, TQ).start()

        @pl.when(jnp.logical_not(fast))
        def _():
            def qproj(i, c):
                r0 = pl.multiple_of(i * 256, 256)
                q = lax.dot_general(pltpu.bitcast(wt_s[0:D // 2, :], BF), x_buf[p, pl.ds(r0, 256), :],
                                    NT_DIMS, preferred_element_type=F32)
                qt_s[:, pl.ds(r0, 256)] = pltpu.bitcast(q.astype(BF), U32)
                return c
            lax.fori_loop(0, S // 256, qproj, 0)
            def tile(j, c):
                q0 = pl.multiple_of(j * TQ, TQ)
                def head(h, c):
                    l0 = pl.multiple_of((h // 8) * 128, 128)
                    r0 = pl.multiple_of(h * 8, 8)
                    qg = pltpu.bitcast(qt_s[pl.ds(pl.multiple_of((h // 8) * 64, 64), 64), pl.ds(q0, TQ)], BF)
                    rows = lax.broadcasted_iota(I32, (128, TQ), 0) // DH
                    w = jnp.where(rows == h % 8, qg.astype(F32), 0.0).astype(BF)
                    s_s[...] = jnp.dot(kf_s[:, pl.ds(l0, 128)].astype(BF), w, preferred_element_type=F32)
                    m = jnp.max(s_s[...], axis=0, keepdims=True)
                    e = jnp.exp2((s_s[...] - m) * QSCALE)
                    lsum = jnp.sum(e, axis=0, keepdims=True)
                    o = jnp.dot(pltpu.bitcast(vt_s[pl.ds(r0, 8), :], BF), e.astype(BF),
                                preferred_element_type=F32)
                    ot_s[0, pl.ds(pl.multiple_of(h * DH, DH), DH), :] = o / lsum
                    return c
                lax.fori_loop(0, H, head, 0)
                oproj(o_natural(0), q0)
                out_copy(p, q0, TQ).start()
                return c
            lax.fori_loop(0, NT, tile, 0)
        return carry

    lax.fori_loop(0, 2, problem, 0)
    for p in range(2):
        out_copy(p, 0, S).wait()


@jax.jit
def pallas_concat_heads__softmax_full_mha__softmax_full_mha__prompt_kernel(
    A_x: jax.Array,
    A_wqkv: jax.Array,
    A_wo: jax.Array,
    B_x: jax.Array,
    B_wqkv: jax.Array,
    B_wo: jax.Array,
):
    any_spec = pl.BlockSpec(memory_space=pl.ANY)
    return pl.pallas_call(
        _kernel,
        out_shape=jax.ShapeDtypeStruct((1, S, 2 * D), BF),
        in_specs=[any_spec] * 6,
        out_specs=any_spec,
        scratch_shapes=[
            pltpu.VMEM((2, S, D), BF),
            pltpu.VMEM((2, D, 3 * D), BF),
            pltpu.VMEM((2, D, D), BF),
            pltpu.VMEM((D, D), U32),
            pltpu.VMEM((S, D), F32),
            pltpu.VMEM((D, 128), F32),
            pltpu.VMEM((H, S // 4, 128), U32),
            pltpu.VMEM((H, 32, S), U32),
            pltpu.VMEM((H, S), F32),
            pltpu.VMEM((D // 2, S), U32),
            pltpu.VMEM((NU, D, TQ), F32),
            pltpu.VMEM((D // 2, S), U32),
            pltpu.VMEM((S, TQ), F32),
            pltpu.VMEM((2, S, D), BF),
            pltpu.SemaphoreType.DMA((2, 4)),
            pltpu.SemaphoreType.DMA((2, len(XCH))),
            pltpu.SemaphoreType.DMA((2,)),
        ],
        compiler_params=pltpu.CompilerParams(vmem_limit_bytes=100 * 1024 * 1024),
        name="mha2",
    )(A_x, A_wqkv, A_wo, B_x, B_wqkv, B_wo)
```

```python
import math

import jax
import jax.numpy as jnp
from jax import lax
import jax.experimental.pallas as pl
import jax.experimental.pallas.tpu as pltpu

S = 2048
D = 512
H = 32
DH = 16
TQ = 128
NT = S // TQ
NU = 2
CH = 256
PT = 128
LT = 13
XCH = (256, 768, 1024)
GS = 2
OP_PREV = ((1, 0), (1, 0), (1, 4), (1, 4))
OP_CUR = (7, 7, 7, 7)
QSCALE = (DH ** -0.5) * math.log2(math.e)
NREP = 6
USPLIT = 6.0
AMAX = 127.0 * (1.0 - 2.0 ** -12)
MAGIC = 1.5 * 2.0 ** 23
RANGE_BOUND = 60.0
PREC_BOUND = 16.0
TINY = 1e-30
BF = jnp.bfloat16
F32 = jnp.float32
I32 = jnp.int32
I8 = jnp.int8
U32 = jnp.uint32
NT_DIMS = (((1,), (1,)), ((), ()))


def _limbs(a):
    th = a + MAGIC
    r = a - (th - MAGIC)
    tu = a * (1.0 / USPLIT) + MAGIC
    tl = r * (NREP * USPLIT) + MAGIC
    return tuple(lax.bitcast_convert_type(t, I32) for t in (th, tu, tl))


def _reduce_rows(xs, op, sub):
    for sh in (1, 2, 4):
        if len(xs) > 1:
            m = (sub & sh) == 0
            xs = [op(jnp.where(m, a, b), pltpu.roll(jnp.where(m, b, a), sh, 0))
                  for a, b in zip(xs[0::2], xs[1::2])]
        else:
            xs = [op(xs[0], pltpu.roll(xs[0], sh, 0))]
    return xs[0]


def _ds(start, size):
    return pl.ds(start if isinstance(start, int) else pl.multiple_of(start, size), size)


def _kernel(ax, aw, ao, bx, bw, bo, out_hbm,
            x_buf, w_buf, wo_buf, wt_s, kf_s, kcol_s, k8_s, q8_s, sc_s, vt_s, ot_s,
            qt_s, s_s, out_buf, w_sem, x_sem, out_sem):
    xoff = [sum(XCH[:i]) for i in range(len(XCH))]

    def w_copy(w, p, part):
        cols = pl.ds(part * D, D)
        return pltpu.make_async_copy(w.at[:, cols], w_buf.at[p, :, cols], w_sem.at[p, part])

    def wo_copy(o, p):
        return pltpu.make_async_copy(o, wo_buf.at[p], w_sem.at[p, 3])

    def x_copy(x, p, i):
        rows = pl.ds(xoff[i], XCH[i])
        return pltpu.make_async_copy(x.at[0, rows, :], x_buf.at[p, rows, :], x_sem.at[p, i])

    def out_copy(p, r0, n):
        return pltpu.make_async_copy(
            out_buf.at[p, pl.ds(r0, n), :],
            out_hbm.at[0, pl.ds(r0, n), _ds(p * D, D)],
            out_sem.at[p])

    w_copy(aw, 0, 1).start()
    x_copy(ax, 0, 0).start()
    x_copy(ax, 0, 1).start()
    ot_s[NU - 1] = jnp.zeros((D, TQ), F32)

    def problem(p, carry):
        w_copy(aw, p, 1).wait()
        kmax = jnp.full((8, D), TINY, F32)
        for i in range(len(XCH)):
            x_copy(ax, p, i).wait()

            @pl.when(p == 0)
            def _():
                if i == 0:
                    x_copy(ax, 0, 2).start()
                    w_copy(aw, 0, 0).start()
                if i == 1:
                    w_copy(aw, 0, 2).start()
                if i == 2:
                    wo_copy(ao, 0).start()
                    for part in (1, 0, 2):
                        w_copy(bw, 1, part).start()
                    for c in range(len(XCH)):
                        x_copy(bx, 1, c).start()
                    wo_copy(bo, 1).start()

            if i == len(XCH) - 1:
                w_copy(aw, p, 0).wait()
            rows = slice(xoff[i], xoff[i] + XCH[i])
            k = jnp.dot(x_buf[p, rows, :], w_buf[p, :, D:2 * D], preferred_element_type=F32)
            kf_s[rows, :] = k
            kmax = jnp.maximum(kmax, jnp.abs(k).reshape(XCH[i] // 8, 8, D).max(axis=0))
        wt_s[0:D // 2, :] = pltpu.bitcast(w_buf[p, :, 0:D].astype(F32).T.astype(BF), U32)
        w_copy(aw, p, 2).wait()
        wt_s[D // 2:D, :] = pltpu.bitcast(w_buf[p, :, 2 * D:3 * D].astype(F32).T.astype(BF), U32)

        kmax = jnp.max(kmax, axis=0, keepdims=True)
        kinv = 127.0 / kmax
        kcol_s[...] = jnp.broadcast_to(kmax * QSCALE, (128, D)).T

        lane_blk = lax.broadcasted_iota(I32, (8, 128), 1) // DH
        masks = [(lane_blk & (1 << b)) != 0 for b in range(3)]
        sub = lax.broadcasted_iota(I32, (8, 128), 0)


        def q_tile(n, c):
            qsm, l1m = c
            cols = _ds(n * 128, 128)
            q = lax.dot_general(pltpu.bitcast(wt_s[0:D // 2, :], BF), x_buf[p, cols, :],
                                NT_DIMS, preferred_element_type=F32)
            for g in range(H // GS):
                rows = slice(g * GS * DH, (g + 1) * GS * DH)
                qp = q[rows] * kcol_s[rows, :]
                aq = jnp.abs(qp)
                lo = [aq[h * DH:h * DH + 8] for h in range(GS)]
                hi = [aq[h * DH + 8:(h + 1) * DH] for h in range(GS)]
                qs = _reduce_rows([jnp.maximum(a, b) for a, b in zip(lo, hi)], jnp.maximum, sub)
                l1 = _reduce_rows([a + b for a, b in zip(lo, hi)], jnp.add, sub)
                qsm = jnp.maximum(qsm, qs)
                l1m = jnp.maximum(l1m, l1)
                qs = jnp.maximum(qs, TINY)
                r = pl.reciprocal(qs, approx=True)
                r = r * (2.0 - qs * r) * AMAX
                sc_s[g * GS:(g + 1) * GS, cols] = (qs * (1.0 / (NREP * AMAX * 127.0)))[0:GS]
                for u in range(GS):
                    h = g * GS + u
                    ah, au, al = _limbs(qp[u * DH:(u + 1) * DH] * r[u:u + 1, :])
                    blocks = []
                    for j in range(8):
                        pair = (j - h) % 8
                        blocks.append(ah if pair < NREP else (au if pair == NREP else al))
                    w8 = jnp.concatenate(blocks, axis=0).astype(I8)
                    q8_s[h, :, cols] = pltpu.bitcast(w8, U32)
            return qsm, l1m
        z = jnp.zeros((8, 128), F32)
        qsm, l1m = lax.fori_loop(0, NT, q_tile, (z, z), unroll=True)

        def v_tile(n, vmax):
            cols = _ds(n * 128, 128)
            v = lax.dot_general(pltpu.bitcast(wt_s[D // 2:D, :], BF), x_buf[p, cols, :],
                                NT_DIMS, preferred_element_type=F32)
            vt_s[:, cols] = pltpu.bitcast(v.astype(BF), U32)
            vmax = jnp.maximum(vmax, jnp.abs(v).reshape(D // 8, 8, 128).max(axis=0))
            bh, bu, bl = [pltpu.bitcast(t.astype(I8), U32)
                          for t in _limbs(kf_s[cols, :] * kinv)]
            for g in range(D // 128):
                pieces = []
                for t in range(4):
                    ys = []
                    for pair in range(8):
                        src = bh if pair < NREP else (bl if pair == NREP else bu)
                        y = src[t * 8:(t + 1) * 8, g * 128:(g + 1) * 128]
                        ys.append(pltpu.roll(y, DH * pair, 1) if pair else y)
                    for b in range(3):
                        ys = [jnp.where(masks[b], ys[(m + (1 << b)) % 8], ys[m]) for m in range(8)]
                    pieces.append(ys)
                for pos in range(8):
                    k8_s[g * 8 + pos, _ds(n * 32, 32), :] = jnp.concatenate(
                        [ys[(8 - pos) % 8] for ys in pieces], axis=0)
            return vmax
        vmax = lax.fori_loop(0, NT, v_tile, z, unroll=True)
        vm = jnp.max(vmax)
        worst = jnp.max(jnp.maximum(l1m * (1.0 / RANGE_BOUND), qsm * (1.0 / PREC_BOUND)))
        fast = jnp.logical_and(worst <= 1.0, jnp.logical_and(vm <= 2.0 ** 40, vm >= 2.0 ** -40))
        wo_copy(ao, p).wait()

        def o_natural(slot):
            return ot_s[slot].T.astype(BF)

        def oproj(o, r0, ns=tuple(range(D // 128))):
            for n in ns:
                out_buf[p, pl.ds(r0, TQ), n * 128:(n + 1) * 128] = jnp.dot(
                    o, wo_buf[p, :, n * 128:(n + 1) * 128], preferred_element_type=F32).astype(BF)

        @pl.when(fast)
        def _():
            nch = S // CH
            tpc = CH // PT
            per = PT // 32
            npt = S // PT
            nunit = NU * H
            order = [t * per + (per - 1 - i) for t in range(tpc) for i in range(per)]
            inv = {b: i for i, b in enumerate(order)}

            def pv(h, t, pt, acc):
                vv = pltpu.bitcast(vt_s[_ds(h * 8, 8), t * PT:(t + 1) * PT], BF)
                o = jnp.dot(vv, pt, preferred_element_type=F32)
                return o if acc is None else acc + o

            def finish(unit, acc, l):
                ot_s[unit // H, _ds((unit % H) * DH, DH), :] = acc / l.sum(axis=0, keepdims=True)

            def body(j, c):
                def unit_step(unit, state, first=False, hook=None):
                    pend, acc_prev, l_prev = state
                    pend = list(pend)
                    h = unit % H
                    qcols = _ds((NU * j + unit // H) * TQ, TQ)
                    w = pltpu.bitcast(q8_s[h, :, qcols], I8)
                    sc = sc_s[pl.ds(h, 1), qcols]
                    l = acc = None
                    done = -LT
                    for c in range(nch):
                        kk = k8_s[h, c * CH // 4:(c + 1) * CH // 4, :]
                        kk = jnp.concatenate([kk[b * 8:(b + 1) * 8] for b in order], axis=0)
                        a = jnp.dot(pltpu.bitcast(kk, I8), w, preferred_element_type=I32)
                        e = jnp.exp2(a.astype(F32) * sc)
                        ls = e.reshape(CH // 8, 8, TQ).sum(axis=0)
                        l = ls if l is None else l + ls
                        for t in range(tpc):
                            et = jnp.concatenate([e[inv[b] * 32:(inv[b] + 1) * 32]
                                                  for b in range(t * per, (t + 1) * per)], axis=0)
                            pend.append(et.astype(BF))
                        if hook is not None:
                            for fn in hook.get(c, ()):
                                fn()
                        for _ in range(tpc):
                            if done >= 0:
                                acc = pv(h, done, pend.pop(0), acc)
                            elif not first:
                                acc_prev = pv((unit - 1) % H, npt + done, pend.pop(0), acc_prev)
                                if done == -1:
                                    finish(unit - 1, acc_prev, l_prev)
                            done += 1
                    return tuple(pend), acc, l

                q0 = pl.multiple_of(NU * j * TQ, TQ)
                prev0 = pl.multiple_of(((NU * j + NT - 1) % NT) * TQ, TQ)
                o_prev = o_natural(NU - 1)
                hooks = {}
                for n, (uu, cc) in enumerate(OP_PREV):
                    hooks.setdefault(uu, {}).setdefault(cc, []).append(
                        lambda n=n: oproj(o_prev, prev0, (n,)))
                last = max(hooks)
                state = unit_step(0, ((), None, None), first=True, hook=hooks.get(0))
                for uu in range(1, last + 1):
                    state = unit_step(uu, state, hook=hooks.get(uu))
                state = lax.fori_loop(last + 1, nunit - 1, unit_step, state, unroll=True)
                o_cur = o_natural(0)
                hook = {}
                for n, cc in enumerate(OP_CUR):
                    hook.setdefault(cc, []).append(lambda n=n: oproj(o_cur, q0, (n,)))
                pend, acc, l = unit_step(nunit - 1, state, hook=hook)
                for i in range(LT):
                    acc = pv(H - 1, npt - LT + i, pend[i], acc)
                finish(nunit - 1, acc, l)

                @pl.when(j > 0)
                def _():
                    out_copy(p, prev0, TQ).start()
                out_copy(p, q0, TQ).start()
                return c
            lax.fori_loop(0, NT // NU, body, 0)
            oproj(o_natural(NU - 1), S - TQ)
            out_copy(p, S - TQ, TQ).start()

        @pl.when(jnp.logical_not(fast))
        def _():
            def qproj(i, c):
                rows = _ds(i * 256, 256)
                q = lax.dot_general(pltpu.bitcast(wt_s[0:D // 2, :], BF), x_buf[p, rows, :],
                                    NT_DIMS, preferred_element_type=F32)
                qt_s[:, rows] = pltpu.bitcast(q.astype(BF), U32)
                return c
            lax.fori_loop(0, S // 256, qproj, 0)

            def tile(j, c):
                q0 = pl.multiple_of(j * TQ, TQ)

                def head(h, c):
                    qg = pltpu.bitcast(qt_s[_ds((h // 8) * 64, 64), pl.ds(q0, TQ)], BF)
                    rows = lax.broadcasted_iota(I32, (128, TQ), 0) // DH
                    w = jnp.where(rows == h % 8, qg.astype(F32), 0.0).astype(BF)
                    s_s[...] = jnp.dot(kf_s[:, _ds((h // 8) * 128, 128)].astype(BF), w,
                                       preferred_element_type=F32)
                    m = jnp.max(s_s[...], axis=0, keepdims=True)
                    e = jnp.exp2((s_s[...] - m) * QSCALE)
                    lsum = jnp.sum(e, axis=0, keepdims=True)
                    o = jnp.dot(pltpu.bitcast(vt_s[_ds(h * 8, 8), :], BF), e.astype(BF),
                                preferred_element_type=F32)
                    ot_s[0, _ds(h * DH, DH), :] = o / lsum
                    return c
                lax.fori_loop(0, H, head, 0)
                oproj(o_natural(0), q0)
                out_copy(p, q0, TQ).start()
                return c
            lax.fori_loop(0, NT, tile, 0)
        return carry

    lax.fori_loop(0, 2, problem, 0)
    for p in range(2):
        out_copy(p, 0, S).wait()


@jax.jit
def pallas_concat_heads__softmax_full_mha__softmax_full_mha__prompt_kernel(
    A_x: jax.Array,
    A_wqkv: jax.Array,
    A_wo: jax.Array,
    B_x: jax.Array,
    B_wqkv: jax.Array,
    B_wo: jax.Array,
):
    any_spec = pl.BlockSpec(memory_space=pl.ANY)
    return pl.pallas_call(
        _kernel,
        out_shape=jax.ShapeDtypeStruct((1, S, 2 * D), BF),
        in_specs=[any_spec] * 6,
        out_specs=any_spec,
        scratch_shapes=[
            pltpu.VMEM((2, S, D), BF),
            pltpu.VMEM((2, D, 3 * D), BF),
            pltpu.VMEM((2, D, D), BF),
            pltpu.VMEM((D, D), U32),
            pltpu.VMEM((S, D), F32),
            pltpu.VMEM((D, 128), F32),
            pltpu.VMEM((H, S // 4, 128), U32),
            pltpu.VMEM((H, 32, S), U32),
            pltpu.VMEM((H, S), F32),
            pltpu.VMEM((D // 2, S), U32),
            pltpu.VMEM((NU, D, TQ), F32),
            pltpu.VMEM((D // 2, S), U32),
            pltpu.VMEM((S, TQ), F32),
            pltpu.VMEM((2, S, D), BF),
            pltpu.SemaphoreType.DMA((2, 4)),
            pltpu.SemaphoreType.DMA((2, len(XCH))),
            pltpu.SemaphoreType.DMA((2,)),
        ],
        compiler_params=pltpu.CompilerParams(vmem_limit_bytes=100 * 1024 * 1024),
        name="mha2",
    )(A_x, A_wqkv, A_wo, B_x, B_wqkv, B_wo)
```

```python
import math

import jax
import jax.numpy as jnp
from jax import lax
import jax.experimental.pallas as pl
import jax.experimental.pallas.tpu as pltpu

S = 2048
D = 512
H = 32
DH = 16
TQ = 128
NT = S // TQ
NU = 2
CH = 256
PT = 128
LT = 13
XCH = (256, 768, 1024)
GS = 2
OP_PREV = ((1, 0), (1, 0), (1, 4), (1, 4))
OP_CUR = (7, 7, 7, 7)
QSCALE = (DH ** -0.5) * math.log2(math.e)
NREP = 6
USPLIT = 6.0
AMAX = 127.0 * (1.0 - 2.0 ** -12)
MAGIC = 1.5 * 2.0 ** 23
RANGE_BOUND = 60.0
PREC_BOUND = 12.0
TINY = 1e-30
BF = jnp.bfloat16
F32 = jnp.float32
I32 = jnp.int32
I8 = jnp.int8
U32 = jnp.uint32
NT_DIMS = (((1,), (1,)), ((), ()))


def _limbs(a):
    th = a + MAGIC
    r = a - (th - MAGIC)
    tu = a * (1.0 / USPLIT) + MAGIC
    tl = r * (NREP * USPLIT) + MAGIC
    return tuple(lax.bitcast_convert_type(t, I32) for t in (th, tu, tl))


def _recip(x):
    r = pl.reciprocal(x, approx=True)
    return r * (2.0 - x * r)


def _reduce_rows(xs, op, sub):
    for sh in (1, 2, 4):
        if len(xs) > 1:
            m = (sub & sh) == 0
            xs = [op(jnp.where(m, a, b), pltpu.roll(jnp.where(m, b, a), sh, 0))
                  for a, b in zip(xs[0::2], xs[1::2])]
        else:
            xs = [op(xs[0], pltpu.roll(xs[0], sh, 0))]
    return xs[0]


def _ds(start, size):
    return pl.ds(start if isinstance(start, int) else pl.multiple_of(start, size), size)


def _kernel(ax, aw, ao, bx, bw, bo, out_hbm,
            x_buf, w_buf, wo_buf, wt_s, kf_s, kcol_s, k8_s, q8_s, sc_s, vt_s, ot_s,
            qt_s, s_s, out_buf, w_sem, x_sem, out_sem):
    xoff = [sum(XCH[:i]) for i in range(len(XCH))]

    def w_copy(w, p, part):
        cols = pl.ds(part * D, D)
        return pltpu.make_async_copy(w.at[:, cols], w_buf.at[p, :, cols], w_sem.at[p, part])

    def wo_copy(o, p):
        return pltpu.make_async_copy(o, wo_buf.at[p], w_sem.at[p, 3])

    def x_copy(x, p, i):
        rows = pl.ds(xoff[i], XCH[i])
        return pltpu.make_async_copy(x.at[0, rows, :], x_buf.at[p, rows, :], x_sem.at[p, i])

    def out_copy(p, r0, n):
        return pltpu.make_async_copy(
            out_buf.at[p, pl.ds(r0, n), :],
            out_hbm.at[0, pl.ds(r0, n), _ds(p * D, D)],
            out_sem.at[p])

    w_copy(aw, 0, 1).start()
    x_copy(ax, 0, 0).start()
    x_copy(ax, 0, 1).start()
    ot_s[NU - 1] = jnp.zeros((D, TQ), F32)

    def problem(p, carry):
        w_copy(aw, p, 1).wait()
        kmax = jnp.full((8, D), TINY, F32)
        for i in range(len(XCH)):
            x_copy(ax, p, i).wait()

            @pl.when(p == 0)
            def _():
                if i == 0:
                    x_copy(ax, 0, 2).start()
                    w_copy(aw, 0, 0).start()
                if i == 1:
                    w_copy(aw, 0, 2).start()
                if i == 2:
                    wo_copy(ao, 0).start()
                    for part in (1, 0, 2):
                        w_copy(bw, 1, part).start()
                    for c in range(len(XCH)):
                        x_copy(bx, 1, c).start()
                    wo_copy(bo, 1).start()

            if i == len(XCH) - 1:
                w_copy(aw, p, 0).wait()
            rows = slice(xoff[i], xoff[i] + XCH[i])
            k = jnp.dot(x_buf[p, rows, :], w_buf[p, :, D:2 * D], preferred_element_type=F32)
            kf_s[rows, :] = k
            kmax = jnp.maximum(kmax, jnp.abs(k).reshape(XCH[i] // 8, 8, D).max(axis=0))
        wt_s[0:D // 2, :] = pltpu.bitcast(w_buf[p, :, 0:D].astype(F32).T.astype(BF), U32)
        w_copy(aw, p, 2).wait()
        wt_s[D // 2:D, :] = pltpu.bitcast(w_buf[p, :, 2 * D:3 * D].astype(F32).T.astype(BF), U32)

        kmax = jnp.max(kmax, axis=0, keepdims=True)
        kinv = 127.0 / kmax
        kcol_s[...] = jnp.broadcast_to(kmax * QSCALE, (128, D)).T

        lane_blk = lax.broadcasted_iota(I32, (8, 128), 1) // DH
        masks = [(lane_blk & (1 << b)) != 0 for b in range(3)]
        sub = lax.broadcasted_iota(I32, (8, 128), 0)


        def q_tile(n, c):
            qsm, l1m = c
            cols = _ds(n * 128, 128)
            q = lax.dot_general(pltpu.bitcast(wt_s[0:D // 2, :], BF), x_buf[p, cols, :],
                                NT_DIMS, preferred_element_type=F32)
            for g in range(H // GS):
                rows = slice(g * GS * DH, (g + 1) * GS * DH)
                qp = q[rows] * kcol_s[rows, :]
                aq = jnp.abs(qp)
                lo = [aq[h * DH:h * DH + 8] for h in range(GS)]
                hi = [aq[h * DH + 8:(h + 1) * DH] for h in range(GS)]
                qs = _reduce_rows([jnp.maximum(a, b) for a, b in zip(lo, hi)], jnp.maximum, sub)
                l1 = _reduce_rows([a + b for a, b in zip(lo, hi)], jnp.add, sub)
                qsm = jnp.maximum(qsm, qs)
                l1m = jnp.maximum(l1m, l1)
                qs = jnp.maximum(qs, TINY)
                r = _recip(qs) * AMAX
                sc_s[g * GS:(g + 1) * GS, cols] = (qs * (1.0 / (NREP * AMAX * 127.0)))[0:GS]
                for u in range(GS):
                    h = g * GS + u
                    ah, au, al = _limbs(qp[u * DH:(u + 1) * DH] * r[u:u + 1, :])
                    blocks = []
                    for j in range(8):
                        pair = (j - h) % 8
                        blocks.append(ah if pair < NREP else (au if pair == NREP else al))
                    w8 = jnp.concatenate(blocks, axis=0).astype(I8)
                    q8_s[h, :, cols] = pltpu.bitcast(w8, U32)
            return qsm, l1m
        z = jnp.zeros((8, 128), F32)
        qsm, l1m = lax.fori_loop(0, NT, q_tile, (z, z), unroll=True)

        def v_tile(n, vmax):
            cols = _ds(n * 128, 128)
            v = lax.dot_general(pltpu.bitcast(wt_s[D // 2:D, :], BF), x_buf[p, cols, :],
                                NT_DIMS, preferred_element_type=F32)
            vt_s[:, cols] = pltpu.bitcast(v.astype(BF), U32)
            vmax = jnp.maximum(vmax, jnp.abs(v).reshape(D // 8, 8, 128).max(axis=0))
            bh, bu, bl = [pltpu.bitcast(t.astype(I8), U32)
                          for t in _limbs(kf_s[cols, :] * kinv)]
            for g in range(D // 128):
                pieces = []
                for t in range(4):
                    ys = []
                    for pair in range(8):
                        src = bh if pair < NREP else (bl if pair == NREP else bu)
                        y = src[t * 8:(t + 1) * 8, g * 128:(g + 1) * 128]
                        ys.append(pltpu.roll(y, DH * pair, 1) if pair else y)
                    for b in range(3):
                        ys = [jnp.where(masks[b], ys[(m + (1 << b)) % 8], ys[m]) for m in range(8)]
                    pieces.append(ys)
                for pos in range(8):
                    k8_s[g * 8 + pos, _ds(n * 32, 32), :] = jnp.concatenate(
                        [ys[(8 - pos) % 8] for ys in pieces], axis=0)
            return vmax
        vmax = lax.fori_loop(0, NT, v_tile, z, unroll=True)
        vm = jnp.max(vmax)
        worst = jnp.max(jnp.maximum(l1m * (1.0 / RANGE_BOUND), qsm * (1.0 / PREC_BOUND)))
        fast = jnp.logical_and(worst <= 1.0, jnp.logical_and(vm <= 2.0 ** 40, vm >= 2.0 ** -40))
        wo_copy(ao, p).wait()

        def o_natural(slot):
            return ot_s[slot].T.astype(BF)

        def oproj(o, r0, ns=tuple(range(D // 128))):
            for n in ns:
                out_buf[p, pl.ds(r0, TQ), n * 128:(n + 1) * 128] = jnp.dot(
                    o, wo_buf[p, :, n * 128:(n + 1) * 128], preferred_element_type=F32).astype(BF)

        @pl.when(fast)
        def _():
            nch = S // CH
            tpc = CH // PT
            per = PT // 32
            npt = S // PT
            nunit = NU * H
            order = [t * per + (per - 1 - i) for t in range(tpc) for i in range(per)]
            inv = {b: i for i, b in enumerate(order)}

            def pv(h, t, pt, acc):
                vv = pltpu.bitcast(vt_s[_ds(h * 8, 8), t * PT:(t + 1) * PT], BF)
                o = jnp.dot(vv, pt, preferred_element_type=F32)
                return o if acc is None else acc + o

            def finish(unit, acc, l):
                ot_s[unit // H, _ds((unit % H) * DH, DH), :] = acc * _recip(
                    l.sum(axis=0, keepdims=True))

            def body(j, c):
                def unit_step(unit, state, first=False, hook=None):
                    pend, acc_prev, l_prev = state
                    pend = list(pend)
                    h = unit % H
                    qcols = _ds((NU * j + unit // H) * TQ, TQ)
                    w = pltpu.bitcast(q8_s[h, :, qcols], I8)
                    sc = sc_s[pl.ds(h, 1), qcols]
                    l = acc = None
                    done = -LT
                    for c in range(nch):
                        kk = k8_s[h, c * CH // 4:(c + 1) * CH // 4, :]
                        kk = jnp.concatenate([kk[b * 8:(b + 1) * 8] for b in order], axis=0)
                        a = jnp.dot(pltpu.bitcast(kk, I8), w, preferred_element_type=I32)
                        e = jnp.exp2(a.astype(F32) * sc)
                        ls = e.reshape(CH // 8, 8, TQ).sum(axis=0)
                        l = ls if l is None else l + ls
                        for t in range(tpc):
                            et = jnp.concatenate([e[inv[b] * 32:(inv[b] + 1) * 32]
                                                  for b in range(t * per, (t + 1) * per)], axis=0)
                            pend.append(et.astype(BF))
                        if hook is not None:
                            for fn in hook.get(c, ()):
                                fn()
                        for _ in range(tpc):
                            if done >= 0:
                                acc = pv(h, done, pend.pop(0), acc)
                            elif not first:
                                acc_prev = pv((unit - 1) % H, npt + done, pend.pop(0), acc_prev)
                                if done == -1:
                                    finish(unit - 1, acc_prev, l_prev)
                            done += 1
                    return tuple(pend), acc, l

                q0 = pl.multiple_of(NU * j * TQ, TQ)
                prev0 = pl.multiple_of(((NU * j + NT - 1) % NT) * TQ, TQ)
                o_prev = o_natural(NU - 1)
                hooks = {}
                for n, (uu, cc) in enumerate(OP_PREV):
                    hooks.setdefault(uu, {}).setdefault(cc, []).append(
                        lambda n=n: oproj(o_prev, prev0, (n,)))
                last = max(hooks)
                state = unit_step(0, ((), None, None), first=True, hook=hooks.get(0))
                for uu in range(1, last + 1):
                    state = unit_step(uu, state, hook=hooks.get(uu))
                state = lax.fori_loop(last + 1, nunit - 1, unit_step, state, unroll=True)
                o_cur = o_natural(0)
                hook = {}
                for n, cc in enumerate(OP_CUR):
                    hook.setdefault(cc, []).append(lambda n=n: oproj(o_cur, q0, (n,)))
                pend, acc, l = unit_step(nunit - 1, state, hook=hook)
                for i in range(LT):
                    acc = pv(H - 1, npt - LT + i, pend[i], acc)
                finish(nunit - 1, acc, l)

                @pl.when(j > 0)
                def _():
                    out_copy(p, prev0, TQ).start()
                out_copy(p, q0, TQ).start()
                return c
            lax.fori_loop(0, NT // NU, body, 0)
            oproj(o_natural(NU - 1), S - TQ)
            out_copy(p, S - TQ, TQ).start()

        @pl.when(jnp.logical_not(fast))
        def _():
            def qproj(i, c):
                rows = _ds(i * 256, 256)
                q = lax.dot_general(pltpu.bitcast(wt_s[0:D // 2, :], BF), x_buf[p, rows, :],
                                    NT_DIMS, preferred_element_type=F32)
                qt_s[:, rows] = pltpu.bitcast(q.astype(BF), U32)
                return c
            lax.fori_loop(0, S // 256, qproj, 0)

            def tile(j, c):
                q0 = pl.multiple_of(j * TQ, TQ)

                def head(h, c):
                    qg = pltpu.bitcast(qt_s[_ds((h // 8) * 64, 64), pl.ds(q0, TQ)], BF)
                    rows = lax.broadcasted_iota(I32, (128, TQ), 0) // DH
                    w = jnp.where(rows == h % 8, qg.astype(F32), 0.0).astype(BF)
                    s_s[...] = jnp.dot(kf_s[:, _ds((h // 8) * 128, 128)].astype(BF), w,
                                       preferred_element_type=F32)
                    m = jnp.max(s_s[...], axis=0, keepdims=True)
                    e = jnp.exp2((s_s[...] - m) * QSCALE)
                    lsum = jnp.sum(e, axis=0, keepdims=True)
                    o = jnp.dot(pltpu.bitcast(vt_s[_ds(h * 8, 8), :], BF), e.astype(BF),
                                preferred_element_type=F32)
                    ot_s[0, _ds(h * DH, DH), :] = o / lsum
                    return c
                lax.fori_loop(0, H, head, 0)
                oproj(o_natural(0), q0)
                out_copy(p, q0, TQ).start()
                return c
            lax.fori_loop(0, NT, tile, 0)
        return carry

    lax.fori_loop(0, 2, problem, 0)
    for p in range(2):
        out_copy(p, 0, S).wait()


@jax.jit
def pallas_concat_heads__softmax_full_mha__softmax_full_mha__prompt_kernel(
    A_x: jax.Array,
    A_wqkv: jax.Array,
    A_wo: jax.Array,
    B_x: jax.Array,
    B_wqkv: jax.Array,
    B_wo: jax.Array,
):
    any_spec = pl.BlockSpec(memory_space=pl.ANY)
    return pl.pallas_call(
        _kernel,
        out_shape=jax.ShapeDtypeStruct((1, S, 2 * D), BF),
        in_specs=[any_spec] * 6,
        out_specs=any_spec,
        scratch_shapes=[
            pltpu.VMEM((2, S, D), BF),
            pltpu.VMEM((2, D, 3 * D), BF),
            pltpu.VMEM((2, D, D), BF),
            pltpu.VMEM((D, D), U32),
            pltpu.VMEM((S, D), F32),
            pltpu.VMEM((D, 128), F32),
            pltpu.VMEM((H, S // 4, 128), U32),
            pltpu.VMEM((H, 32, S), U32),
            pltpu.VMEM((H, S), F32),
            pltpu.VMEM((D // 2, S), U32),
            pltpu.VMEM((NU, D, TQ), F32),
            pltpu.VMEM((D // 2, S), U32),
            pltpu.VMEM((S, TQ), F32),
            pltpu.VMEM((2, S, D), BF),
            pltpu.SemaphoreType.DMA((2, 4)),
            pltpu.SemaphoreType.DMA((2, len(XCH))),
            pltpu.SemaphoreType.DMA((2,)),
        ],
        compiler_params=pltpu.CompilerParams(vmem_limit_bytes=100 * 1024 * 1024),
        name="mha2",
    )(A_x, A_wqkv, A_wo, B_x, B_wqkv, B_wo)
```
